```python
import os as _os
_os.environ.setdefault("JAX_PLATFORMS", "cpu")
import jax
import jax.numpy as jnp

def _softmax(x, axis=-1):
    return jax.nn.softmax(x, axis=axis)
def _gelu(x):
    return jax.nn.gelu(x, approximate=True)
def _silu(x):
    return jax.nn.silu(x)
def _sigmoid(x):
    return jax.nn.sigmoid(x)
def _layernorm(x, axis=-1, eps=1e-5):
    m = jnp.mean(x, axis=axis, keepdims=True)
    v = jnp.var(x, axis=axis, keepdims=True)
    return (x - m) / jnp.sqrt(v + eps)
def _scatter_add(tgt, idx, src, axis=0):
    return tgt.at[idx].add(src)
def _segment_sum(src, seg, n):
    return jax.ops.segment_sum(src, seg, n)
class _Rng:
    def __init__(self, key):
        self._k = key
    def _next(self):
        self._k, sub = jax.random.split(self._k)
        return sub
    def normal(self, shape):
        return jax.random.normal(self._next(), shape, dtype=jnp.bfloat16)
    def randint(self, lo, hi, shape):
        return jax.random.randint(self._next(), shape, lo, hi, dtype=jnp.int32)
    def uniform(self, shape, lo=0.0, hi=1.0):
        return jax.random.uniform(self._next(), shape, jnp.bfloat16, lo, hi)
    def permutation(self, n):
        return jax.random.permutation(self._next(), n)


kernel_name = 'interleave_layers__sliding_local_dilated__moe_arch_mod__prompt'

def setup_inputs():
    _rng = _Rng(jax.random.key(int.from_bytes(__import__("os").urandom(4), "little")))
    _w = (lambda a: (lambda t: t.astype(jnp.bfloat16) if jnp.issubdtype(t.dtype, jnp.floating) else t)(jnp.asarray(a)))
    def _A_setup():
        B, S, D = 1, 2048, 512
        return {
            "x": _w((lambda *s: _rng.normal(s) * 0.05)(B, S, D)),
            "wqkv": _w((lambda *s: _rng.normal(s) * 0.05)(D, 3 * D)),
            "wo": _w((lambda *s: _rng.normal(s) * 0.05)(D, D)),
        }
    _A_in = _A_setup()

    def _B_setup():
        B, S, D, F, C = 1, 2048, 512, 1376, 2
        return {
            "x": _w((lambda *s: _rng.normal(s) * 0.05)(B, S, D)),
            "w_r": _w((lambda *s: _rng.normal(s) * 0.05)(D)),
            "w_gate": _w((lambda *s: _rng.normal(s) * 0.05)(D, F)),
            "w_up": _w((lambda *s: _rng.normal(s) * 0.05)(D, F)),
            "w_down": _w((lambda *s: _rng.normal(s) * 0.05)(F, D)),
        }
    _B_in = _B_setup()

    return {
        "A_x": _A_in["x"],
        "A_wqkv": _A_in["wqkv"],
        "A_wo": _A_in["wo"],
        "B_x": _B_in["x"],
        "B_w_r": _B_in["w_r"],
        "B_w_gate": _B_in["w_gate"],
        "B_w_up": _B_in["w_up"],
        "B_w_down": _B_in["w_down"],
    }

def reference(A_x, A_wqkv, A_wo, B_x, B_w_r, B_w_gate, B_w_up, B_w_down):
    def _A_ref(x, wqkv, wo):
        B, S, D = x.shape
        H = 32; Dh = D // H
        W, dil = 8, 2
        qkv = (lambda x, *d: x.transpose(*d))((x @ wqkv).reshape(B, S, 3, H, Dh), 2, 0, 3, 1, 4)
        q, k, v = qkv[0], qkv[1], qkv[2]
        scale = Dh ** -0.5
        pos = jnp.arange(S)
        off = jnp.arange(W) * dil
        idx = pos[:, None] - off[None, :]
        mask = idx >= 0
        idx_c = jnp.where(mask, idx, 0).reshape(-1)
        kg = k[:, :, idx_c, :].reshape(B, H, S, W, Dh)
        vg = v[:, :, idx_c, :].reshape(B, H, S, W, Dh)
        logits = jnp.einsum("bhsd,bhswd->bhsw", q, kg) * scale
        logits = jnp.where(mask[None, None, :, :], logits, -1e9)
        attn = _softmax(logits, axis=-1)
        o = jnp.einsum("bhsw,bhswd->bhsd", attn, vg)
        return (lambda x, *d: x.transpose(*d))(o, 0, 2, 1, 3).reshape(B, S, D) @ wo

    def _B_ref(x, w_r, w_gate, w_up, w_down):
        B, S, D = x.shape
        C = 2
        r = x @ w_r
        idx = jnp.argsort(-r, axis=-1)[:, :C]
        idx_e = jnp.repeat(idx.reshape(B, C, 1), D, axis=2)
        x_sel = jnp.take_along_axis(x, idx_e, axis=1)
        g = _silu(x_sel @ w_gate)
        u = x_sel @ w_up
        y = (g * u) @ w_down
        r_sel = _sigmoid(jnp.take_along_axis(r, idx, axis=1))
        y = y * r_sel.reshape(B, C, 1)
        b_off = (jnp.arange(B) * S).reshape(B, 1)
        flat_idx = (idx + b_off).reshape(B * C)
        zero = (x * 0.0).reshape(B * S, D)
        upd = _scatter_add(zero, flat_idx, y.reshape(B * C, D), axis=0)
        return x + upd.reshape(B, S, D)

    x = A_x
    x = x + _A_ref(_layernorm(x, axis=-1), A_wqkv, A_wo)
    x = x + _B_ref(_layernorm(x, axis=-1), B_w_r, B_w_gate, B_w_up, B_w_down)
    x = x + _A_ref(_layernorm(x, axis=-1), A_wqkv, A_wo)
    x = x + _B_ref(_layernorm(x, axis=-1), B_w_r, B_w_gate, B_w_up, B_w_down)
    return x
```

```python
import functools
import numpy as np
import jax
import jax.numpy as jnp
from jax import lax
import jax.experimental.pallas as pl
import jax.experimental.pallas.tpu as pltpu

S, D, F = 2048, 512, 1376
NC = 16
W = 8
EPS = 1e-5
F32, BF16, I32, U32 = jnp.float32, jnp.bfloat16, jnp.int32, jnp.uint32
NT = (((1,), (1,)), ((), ()))
NN = (((1,), (0,)), ((), ()))


def _dot(a, b, dn=NN):
    return lax.dot_general(a, b, dn, preferred_element_type=F32)


def _kernel(x_hbm, wqkv_hbm, wo_hbm, wr_ref, wg_hbm, wu_hbm, wd_hbm, out_hbm,
            xin, wqkv, wo, wg, wu, wd, wT, woT, wrB, tbuf,
            xT, hT, qT, kT, vT, oT, stat, rbuf, obuf, sems):
    cp_w = pltpu.make_async_copy(wqkv_hbm, wqkv, sems.at[0])
    cp_x = [pltpu.make_async_copy(x_hbm.at[:, a], xin.at[a], sems.at[1 + a]) for a in range(2)]
    cp_wo = pltpu.make_async_copy(wo_hbm, wo, sems.at[3])
    cp_g = pltpu.make_async_copy(wg_hbm, wg, sems.at[4])
    cp_u = pltpu.make_async_copy(wu_hbm, wu, sems.at[5])
    cp_d = pltpu.make_async_copy(wd_hbm, wd, sems.at[6])
    cp_w.start(); cp_x[1].start(); cp_x[0].start(); cp_wo.start()
    cp_g.start(); cp_u.start(); cp_d.start()

    lane = lax.broadcasted_iota(I32, (8, 128), 1)
    ri = lax.broadcasted_iota(I32, (128, 128), 0)
    ci = lax.broadcasted_iota(I32, (128, 128), 1)
    pm = ci == (ri % 8) * 16 + ri // 8
    P = jnp.where(pm, 1.0, 0.0).astype(BF16)
    Pq = jnp.where(pm, 0.25, 0.0).astype(BF16)

    wrB[...] = jnp.broadcast_to(wr_ref[...].astype(F32).reshape(1, D), (128, D)).T

    cp_w.wait()
    for t in range(12):
        wT[t * 128:(t + 1) * 128, :] = _dot(Pq if t < 4 else P, wqkv[:, t * 128:(t + 1) * 128], NT).astype(BF16)

    def colsum(load):
        acc = load(0)
        for i in range(1, 64):
            acc = acc + load(i)
        return jnp.sum(acc, axis=0, keepdims=True)

    def rows(i, n=8):
        return slice(i * n, (i + 1) * n)

    def ln_col(c):
        m = colsum(lambda i: xT[c, rows(i), :]) * (1.0 / D)
        def sq(i):
            xc = xT[c, rows(i), :] - m
            return xc * xc
        var = colsum(sq) * (1.0 / D)
        rs = lax.rsqrt(var + EPS)
        for i in range(32):
            hT[c, rows(i, 16), :] = ((xT[c, rows(i, 16), :] - m) * rs).astype(BF16)

    def load_x(a):
        cp_x[a].wait()
        for j in range(4):
            for l in range(64):
                tbuf[j, rows(l), :] = pltpu.bitcast(xin[a, l, :, j * 128:(j + 1) * 128], U32)
        for i in range(8):
            c = 8 * a + i
            for j in range(4):
                u = tbuf[j, pl.ds(i, 64, stride=8), :]
                xT[c, j * 128:(j + 1) * 128, :] = pltpu.bitcast(u, BF16).T.astype(F32)
            ln_col(c)

    def proj_q(c):
        qT[c] = _dot(wT[0:512, :], hT[c])

    def proj_kv(c):
        h = hT[c]
        kT[c + 7] = _dot(wT[512:1024, :], h)
        vT[c + 7] = _dot(wT[1024:1536, :], h)

    def wrap(c):
        for i in range(64):
            kT[c - 9, rows(i), :] = pltpu.roll(kT[c + 7, rows(i), :], 2, 1)
            v0 = vT[7, rows(i), :]
            v0 = jnp.where(lane == 0, v0, pltpu.roll(v0, 1, 1))
            vT[c - 9, rows(i), :] = jnp.where(lane < 2, v0, pltpu.roll(vT[c + 7, rows(i), :], 2, 1))

    def attn(c, nmask):
        for g in range(4):
            acc = [None] * W
            for d in range(16):
                r = rows(g * 16 + d)
                q = qT[c, r, :]
                for w in range(W):
                    p = q * kT[c + 7 - w, r, :]
                    acc[w] = p if d == 0 else acc[w] + p
            for w in range(nmask, W):
                acc[w] = jnp.where(lane < 2, -1e9, acc[w])
            mx = acc[0]
            for w in range(1, W):
                mx = jnp.maximum(mx, acc[w])
            e = [jnp.exp(a - mx) for a in acc]
            sm = e[0]
            for w in range(1, W):
                sm = sm + e[w]
            inv = 1.0 / sm
            p = [a * inv for a in e]
            for d2 in range(8):
                o = []
                for d in (2 * d2, 2 * d2 + 1):
                    r = rows(g * 16 + d)
                    t = p[0] * vT[c + 7, r, :]
                    for w in range(1, W):
                        t = t + p[w] * vT[c + 7 - w, r, :]
                    o.append(t)
                oT[c, rows(g * 8 + d2, 16), :] = jnp.concatenate(o, axis=0).astype(BF16)

    def emit(c, i):
        for j in range(4):
            t = xT[c, j * 128:(j + 1) * 128, :].astype(BF16).T
            tbuf[j, pl.ds(i, 64, stride=8), :] = pltpu.bitcast(t, U32)

    def flush(a):
        for j in range(4):
            for l in range(64):
                obuf[a, l, :, j * 128:(j + 1) * 128] = pltpu.bitcast(tbuf[j, rows(l), :], BF16)

    def out_proj(c, last):
        x1 = xT[c] + _dot(woT[...], oT[c])
        xT[c] = x1
        m = colsum(lambda i: xT[c, rows(i), :]) * (1.0 / D)
        va = None
        ra = None
        for i in range(64):
            xc = xT[c, rows(i), :] - m
            va = xc * xc if va is None else va + xc * xc
            t = xc * wrB[rows(i), :]
            ra = t if ra is None else ra + t
        var = jnp.sum(va, axis=0, keepdims=True) * (1.0 / D)
        rs = lax.rsqrt(var + EPS)
        rbuf[pl.ds(c, 1), :] = jnp.sum(ra, axis=0, keepdims=True) * rs
        g = 1.0 + rs
        stat[0, pl.ds(c, 1), :] = m
        stat[1, pl.ds(c, 1), :] = rs / g
        sc2 = g * lax.rsqrt(var * g * g + EPS)
        for i in range(32):
            x = xT[c, rows(i, 16), :]
            xc = x - m
            xT[c, rows(i, 16), :] = x + xc * rs
            if not last:
                hT[c, rows(i, 16), :] = (xc * sc2).astype(BF16)

    def route(last):
        r = rbuf[...]
        r = jnp.where(r == r, r, -jnp.inf)
        cc = lax.broadcasted_iota(I32, (NC, 128), 0)
        ll = lax.broadcasted_iota(I32, (NC, 128), 1)
        pos = ((ll // 2) * 32 + 2 * cc + ll % 2).astype(F32)
        big = float(S)
        m0 = jnp.max(r, keepdims=True)
        p0 = jnp.min(jnp.where(r == m0, pos, big), keepdims=True)
        r1 = jnp.where(pos == p0, -jnp.inf, r)
        m1 = jnp.max(r1, keepdims=True)
        p1 = jnp.min(jnp.where((r1 == m1) & (pos != p0), pos, big), keepdims=True)
        idx = [jnp.min(p).astype(I32) for p in (p0, p1)]
        cs = [(p % 32) // 2 for p in idx]
        ls = [(p // 32) * 2 + p % 2 for p in idx]
        row16 = lax.broadcasted_iota(I32, (16, 128), 0)
        lane512 = lax.broadcasted_iota(I32, (D, 128), 1)
        sel = None
        for i in range(2):
            h = (xT[cs[i]] - stat[0, pl.ds(cs[i], 1), :]) * stat[1, pl.ds(cs[i], 1), :]
            h = jnp.where(lane512 == ls[i], h, 0.0).astype(BF16)
            t = _dot(jnp.where(row16 == i, 1.0, 0.0).astype(BF16), h, NT)
            sel = t if sel is None else sel + t
        sel = sel.astype(BF16)
        gt = _dot(sel, wg[...], NT)
        up = _dot(sel, wu[...], NT)
        act = (gt * jax.nn.sigmoid(gt) * up).astype(BF16)
        y = _dot(act, wd[...])
        for i, mi in enumerate((m0, m1)):
            yi = y[i:i + 1, :] * jax.nn.sigmoid(mi)
            yb = jnp.broadcast_to(yi, (128, D)).T
            xc = xT[cs[i]]
            xT[cs[i]] = jnp.where(lane512 == ls[i], xc + yb, xc)
        if not last:
            for i in range(2):
                ln_col(cs[i])

    load_x(1)
    load_x(0)
    cp_wo.wait()
    woT_nat = wo[...].T
    for g in range(4):
        woT[:, g * 128:(g + 1) * 128] = _dot(woT_nat[:, g * 128:(g + 1) * 128], P, NT).astype(BF16)

    for layer in range(2):
        last = layer == 1
        proj_kv(0)
        for c in range(9, 16):
            proj_kv(c)
            wrap(c)
        proj_q(0)
        for s in range(NC + 1):
            if s + 1 < NC:
                proj_q(s + 1)
                if s + 1 < 9:
                    proj_kv(s + 1)
            if s < NC:
                attn(s, min(s + 1, W))
            if s >= 1:
                out_proj(s - 1, last)
        if layer == 0:
            cp_g.wait(); cp_u.wait(); cp_d.wait()
        route(last)

    for a in range(2):
        for i in range(8):
            emit(8 * a + i, i)
        flush(a)
    cp_o = [pltpu.make_async_copy(obuf.at[a], out_hbm.at[:, a], sems.at[1 + a]) for a in range(2)]
    for c in cp_o:
        c.start()
    for c in cp_o:
        c.wait()


@jax.jit
def pallas_interleave_layers__sliding_local_dilated__moe_arch_mod__prompt_kernel(
        A_x, A_wqkv, A_wo, B_x, B_w_r, B_w_gate, B_w_up, B_w_down):
    del B_x
    x = A_x.reshape(64, 2, 16, D)
    any_spec = pl.BlockSpec(memory_space=pltpu.HBM)
    out = pl.pallas_call(
        _kernel,
        out_shape=jax.ShapeDtypeStruct((64, 2, 16, D), BF16),
        in_specs=[any_spec, any_spec, any_spec, pl.BlockSpec(memory_space=pltpu.VMEM), any_spec, any_spec, any_spec],
        out_specs=any_spec,
        scratch_shapes=[
            pltpu.VMEM((2, 64, 16, D), BF16),
            pltpu.VMEM((D, 3 * D), BF16),
            pltpu.VMEM((D, D), BF16),
            pltpu.VMEM((F, D), BF16),
            pltpu.VMEM((F, D), BF16),
            pltpu.VMEM((F, D), BF16),
            pltpu.VMEM((3 * D, D), BF16),
            pltpu.VMEM((D, D), BF16),
            pltpu.VMEM((D, 128), F32),
            pltpu.VMEM((4, 512, 128), U32),
            pltpu.VMEM((NC, D, 128), F32),
            pltpu.VMEM((NC, D, 128), BF16),
            pltpu.VMEM((NC, D, 128), F32),
            pltpu.VMEM((NC + 7, D, 128), F32),
            pltpu.VMEM((NC + 7, D, 128), F32),
            pltpu.VMEM((NC, D, 128), BF16),
            pltpu.VMEM((2, NC, 128), F32),
            pltpu.VMEM((NC, 128), F32),
            pltpu.VMEM((2, 64, 16, D), BF16),
            pltpu.SemaphoreType.DMA((7,)),
        ],
        compiler_params=pltpu.CompilerParams(vmem_limit_bytes=100 * 1024 * 1024),
    )(x, A_wqkv, A_wo, B_w_r, B_w_gate.T, B_w_up.T, B_w_down)
    return out.reshape(1, S, D)
```

```python
import jax
import jax.numpy as jnp
from jax import lax
import jax.experimental.pallas as pl
import jax.experimental.pallas.tpu as pltpu

S, D, F = 2048, 512, 1376
NC = 16
NG = 4
W = 8
FT = 11
EPS = 1e-5
SCALE = 0.25
F32, BF16, I32, U32 = jnp.float32, jnp.bfloat16, jnp.int32, jnp.uint32
NN = (((1,), (0,)), ((), ()))
NT = (((1,), (1,)), ((), ()))
K_, V_, Q_ = 0, 1, 2

KV_ORDER = [0] + list(range(9, 16)) + list(range(1, 9))
AT_ORDER = list(range(16))
KV_ORDER0 = [0, 1, 2, 3, 12, 13, 14, 15, 11, 10, 9, 8, 4, 5, 6, 7]
AT_ORDER0 = [3, 2, 1, 0, 15, 4, 5, 6, 7, 8, 9, 10, 11, 12, 13, 14]
LAG = 7
X_STEPS = (0, 2, 7)
W_STEP = 15
FFN_COL = 13
RUN_AHEAD = (3, 1, 1, 3)


def _dot(a, b, dn=NN):
    return lax.dot_general(a, b, dn, preferred_element_type=F32)


def _bf(words):
    return pltpu.bitcast(words, BF16)


def _rows(i, n=8):
    return slice(i * n, (i + 1) * n)


def _tree(op, xs):
    while len(xs) > 1:
        xs = [op(xs[i], xs[i + 1]) for i in range(0, len(xs), 2)]
    return xs[0]


def _start(copies):
    for c in copies:
        c.start()


def _wait(copies):
    for c in copies:
        c.wait()


def _kernel(x_hbm, wqkv_hbm, wo_hbm, wr_hbm, wg_hbm, wu_hbm, wd_hbm, out_hbm,
            xin, wqkv, wo, wr, wr_spare, wg, wu, wd,
            wtmp, wT, woT, womu, omean, wrB, wgu, wdn, tin, tout,
            xa, xb, hT, qT, kT, vT, v0T, oT, stat, rstd, score, obuf, pbuf, sems):
    copy = pltpu.make_async_copy
    cp_w = [[copy(wqkv_hbm.at[:, _rows(p * NG + g, 128)], wqkv.at[p * NG + g], sems.at[g])
             for p in range(3)] for g in range(NG)]
    cp_x = [copy(x_hbm.at[:, a], xin.at[a], sems.at[4 + a]) for a in range(4)]
    cp_wo = [copy(wo_hbm, wo, sems.at[8]), copy(wr_hbm, wr, sems.at[9])]
    cp_ffn = [copy(wg_hbm, wg, sems.at[10]), copy(wu_hbm, wu, sems.at[11]), copy(wd_hbm, wd, sems.at[12])]
    cp_spare = [copy(wr_hbm, wr_spare, sems.at[13])]
    cp_out = [[copy(obuf.at[a, j], out_hbm.at[:, a, :, _rows(j, 128)], sems.at[a])
               for j in range(4)] for a in range(4)]
    _start([cp_x[0]] + cp_w[0] + [cp_x[3], cp_x[2], cp_x[1]])

    lane = lax.broadcasted_iota(I32, (8, 128), 1)
    sub = lax.broadcasted_iota(I32, (8, 128), 0)

    every = lane >= 0

    def put(ref, idx, i, val):
        pltpu.store(ref.at[(*idx, pl.ds(i * 8, 8), slice(None))], val, mask=every)

    def channel_major(slot, t):
        wtmp[slot] = pltpu.bitcast(t, U32)
        out = []
        for i in range(8):
            u = wtmp[slot, pl.ds(i, 8, stride=8), :]
            out += [pltpu.bitcast(u << 16, F32), pltpu.bitcast((u >> 16) << 16, F32)]
        return jnp.concatenate(out, axis=0)

    def prep_wqkv(g):
        for p, part in enumerate((Q_, K_, V_)):
            t = _bf(wqkv.bitcast(U32)[p * NG + g]).T
            for j in range(4):
                u = channel_major(16 + 12 * g + 4 * p + j, t[:, _rows(j, 128)])
                wT[g, j, _rows(part, 128), :] = (u * SCALE if part == Q_ else u).astype(BF16)

    def prep_wo():
        wrB[...] = jnp.broadcast_to(wr[...].astype(F32).reshape(1, D), (128, D)).T
        for g in range(NG):
            t = [channel_major(4 * g + j, wo[_rows(g, 128), _rows(j, 128)]) for j in range(4)]
            mu = jnp.sum(_tree(jnp.add, t), axis=1, keepdims=True) * (1.0 / D)
            for j in range(4):
                woT[g, _rows(j, 128), :] = (t[j] - mu).astype(BF16).T
            womu[g] = jnp.broadcast_to(mu, (128, 128))

    def prep_ffn():
        for t in range(FT):
            n = min(128, F - t * 128)
            for i, w in enumerate((wg, wu)):
                a = w[t * 128:t * 128 + n, :]
                if n < 128:
                    a = jnp.concatenate([a, jnp.zeros((128 - n, D), BF16)], axis=0)
                wgu[:, _rows(2 * t + i, 128)] = pltpu.bitcast(a.T, U32)
            wdn[t * 64:t * 64 + n // 2, :] = pltpu.bitcast(wd[t * 128:t * 128 + n, :], U32)
        wdn[F // 2:, :] = jnp.zeros((FT * 64 - F // 2, D), U32)

    def norm_column(c, x, mean0, dst):
        acc = [x[0], x[1]]
        for i in range(2, 64):
            acc[i % 2] = acc[i % 2] + x[i]
        m = jnp.sum(acc[0] + acc[1], axis=0, keepdims=True) * (1.0 / D)
        for i in range(64):
            t = x[i] - m
            put(dst, (c,), i, t)
            acc[i % 2] = t * t if i < 2 else acc[i % 2] + t * t
        var = jnp.sum(acc[0] + acc[1], axis=0, keepdims=True) * (1.0 / D)
        stat[c] = jnp.where(sub == 0, m if mean0 is None else mean0 + m, 1.0)
        rs = lax.rsqrt(var + EPS)
        for i in range(32):
            hT[c, _rows(i, 16), :] = (dst[c, _rows(i, 16), :] * rs).astype(BF16)

    def stage_x(a):
        for j in range(4):
            tin[a, j] = pltpu.bitcast(xin[a, :, :, _rows(j, 128)].reshape(512, 128), U32)

    def load_column(c):
        x = []
        for j in range(4):
            t = _bf(tin[c // 4, j, pl.ds(c % 4, 64, stride=4), :]).T.astype(F32)
            x += [t[_rows(i)] for i in range(16)]
        norm_column(c, x, None, xa)

    def project(g, c, part=None):
        rr = _rows(0, 128) if part is None else _rows(part, 64)
        w = jnp.concatenate([wT.bitcast(U32)[g, j, rr, :] for j in range(4)], axis=1)
        return _dot(_bf(w), _bf(hT.bitcast(U32)[c]))

    def keep_kv(g, c, r):
        b = g % 2
        for i in range(16):
            k = r[_rows(i)]
            put(kT, (b, c + 7), i, k)
            if c >= 9:
                put(kT, (b, c - 9), i, pltpu.roll(k, 2, 1))
        for i in range(16):
            v = r[_rows(16 + i)]
            put(vT, (b, c + 7), i, v)
            if c == 0:
                v0T[b, _rows(i), :] = jnp.where(lane == 0, v, pltpu.roll(v, 1, 1))
            if c >= 9:
                put(vT, (b, c - 9), i, jnp.where(lane < 2, v0T[b, _rows(i), :], pltpu.roll(v, 2, 1)))

    def keep_q(g, c):
        qT[g % 2, c] = project(g, c, Q_)

    def attend(g, c, with_mean):
        b = g % 2
        logit = [None] * W
        for d in range(16):
            q = qT[b, c, _rows(d), :]
            for w in range(W):
                t = q * kT[b, c + 7 - w, _rows(d), :]
                logit[w] = t if d == 0 else logit[w] + t
        for w in range(c + 1, W):
            logit[w] = jnp.where(lane < 2, -1e9, logit[w])
        top = _tree(jnp.maximum, logit)
        e = [jnp.exp(a - top) for a in logit]
        inv = 1.0 / _tree(jnp.add, e)
        for i in range(8):
            o = []
            for d in (2 * i, 2 * i + 1):
                t = e[0] * vT[b, c + 7, _rows(d), :]
                for w in range(1, W):
                    t = t + e[w] * vT[b, c + 7 - w, _rows(d), :]
                o.append(t * inv)
                if with_mean:
                    u = o[-1] * womu[g, _rows(d), :]
                    shift = u if d == 0 else shift + u
            oT[c, _rows(g * 8 + i, 16), :] = jnp.concatenate(o, axis=0).astype(BF16)
        if with_mean:
            omean[g, c] = shift

    def out_proj(c, last, pending):
        w = jnp.concatenate([woT.bitcast(U32)[j] for j in range(4)], axis=1)
        r = _dot(_bf(w), _bf(oT.bitcast(U32)[c]))
        st = stat[c]
        sq = dot = None
        for i in range(64):
            if last:
                t = xb[c, _rows(i), :] * st[1:2] + r[_rows(i)]
                xa[c, _rows(i), :] = t
            else:
                t = xa[c, _rows(i), :] + r[_rows(i)]
                xb[c, _rows(i), :] = t
            u = t * wrB[_rows(i), :]
            sq = t * t if i == 0 else sq + t * t
            dot = u if i == 0 else dot + u
        var = jnp.sum(sq, axis=0, keepdims=True) * (1.0 / D)
        shift = _tree(jnp.add, [omean[g, c] for g in range(NG)])
        mean = st[0:1] + jnp.sum(shift, axis=0, keepdims=True)
        if pending is None:
            rs = lax.rsqrt(var + EPS)
        else:
            both = lax.rsqrt(jnp.where(sub == 0, var, pending) + EPS)
            rs, pending = both[0:1], both[1:2]
        score[pl.ds(c, 1), :] = jnp.sum(dot, axis=0, keepdims=True) * rs
        rstd[pl.ds(c, 1), :] = rs
        gain = 1.0 + rs
        if last:
            return gain, mean, None
        stat[c] = jnp.where(sub == 0, mean, gain)
        return gain, var * gain * gain, pending

    def next_norm(c, scale):
        for i in range(32):
            hT[c, _rows(i, 16), :] = (xb[c, _rows(i, 16), :] * scale).astype(BF16)

    def emit(c, gain, mean):
        for j in range(4):
            x = xa[c, _rows(j, 128), :] * gain + mean
            tout[c // 4, j, pl.ds(c % 4, 64, stride=4), :] = pltpu.bitcast(x.astype(BF16).T, U32)

    def flush(a):
        for j in range(4):
            obuf.bitcast(U32)[a, j] = tout[a, j].reshape(64, 4, 128)

    def route(last):
        early = {}

        def run_ahead(n):
            for _ in range(0 if last else n):
                c = KV_ORDER[len(early)]
                early[c] = project(0, c)

        r = score[...]
        cc = lax.broadcasted_iota(I32, (NC, 128), 0)
        ll = lax.broadcasted_iota(I32, (NC, 128), 1)
        pos = (ll // 2) * 32 + 2 * cc + ll % 2
        neg = jnp.logical_not(r >= 0.0)
        mag = jnp.clip(pltpu.bitcast(r, I32) & 0x7FFFFFFF, 0x00800000, 0x7F7FFFFF) & ~(S - 1)
        key = pltpu.bitcast(mag | jnp.where(neg, pos, S - 1 - pos), F32)
        key = jnp.where(neg, -key, key)
        k0 = jnp.max(key, keepdims=True)
        k1 = jnp.max(jnp.where(key == k0, -jnp.inf, key), keepdims=True)
        idx = []
        for k in (k0, k1):
            low = pltpu.bitcast(jnp.broadcast_to(k, (8, 128)), I32) & (S - 1)
            idx.append(jnp.where(k < 0.0, low, S - 1 - low)[0, 0])
        cs = [(p >> 1) & (NC - 1) for p in idx]
        ls = [((p >> 5) << 1) | (p & 1) for p in idx]
        rsel = [jnp.sum(jnp.where(lane[0:1] == ls[i], score[pl.ds(cs[i], 1), :], 0.0), keepdims=True)
                for i in range(2)]

        row = lax.broadcasted_iota(I32, (16, 128), 0)
        lanes = lax.broadcasted_iota(I32, (D, 128), 1)
        run_ahead(RUN_AHEAD[0])
        sel = []
        for i in range(2):
            h = (xa if last else xb)[cs[i]] * rstd[pl.ds(cs[i], 1), :]
            h = jnp.where(lanes == ls[i], h, 0.0).astype(BF16)
            sel.append(_dot(jnp.where(row == i, 1.0, 0.0).astype(BF16), h, NT))
        sel = jnp.where(lax.broadcasted_iota(I32, (16, D), 0) == 0, sel[0], sel[1]).astype(BF16)
        if last:
            flush(3)
            _start(cp_out[3])
            _wait(cp_out[0])
        run_ahead(RUN_AHEAD[1])
        gu = _dot(sel, _bf(wgu[...]))[0:8]
        act = []
        for t in range(FT):
            gate = gu[:, _rows(2 * t, 128)]
            act.append(gate * jax.nn.sigmoid(gate) * gu[:, _rows(2 * t + 1, 128)])
        act = jnp.concatenate(act, axis=1)
        act = jnp.concatenate([act, jnp.zeros_like(act)], axis=0).astype(BF16)
        run_ahead(RUN_AHEAD[2])
        y = _dot(act, _bf(wdn[...]))
        run_ahead(RUN_AHEAD[3])
        ys = [y[i:i + 1, :] * jax.nn.sigmoid(rsel[i]) for i in range(2)]

        if not last:
            for i in range(2):
                upd = jnp.broadcast_to(ys[i], (128, D)).astype(BF16).T.astype(F32)
                st = stat[cs[i]]
                x = xb[cs[i]] * st[1:2]
                x = jnp.where(lanes == ls[i], x + upd, x)
                norm_column(cs[i], [x[_rows(k)] for k in range(64)], st[0:1], xb)
            redo = [project(0, cs[i]) for i in range(2)]
            for c, r in early.items():
                keep_kv(0, c, jnp.where(cs[0] == c, redo[0], jnp.where(cs[1] == c, redo[1], r)))
            return len(early)

        grp = [p >> 3 for p in idx]
        grp[1] = jnp.where(grp[0] == grp[1], grp[0] ^ 1, grp[1])
        for i in range(2):
            for j in range(4):
                t = obuf[grp[i] & 3, j, grp[i] >> 2].astype(F32)
                for k in range(2):
                    t = jnp.where(sub + grp[i] * 8 == idx[k], t + ys[k][:, _rows(j, 128)], t)
                pbuf[i, :, _rows(j, 128)] = t.astype(BF16)
        _wait(cp_out[1] + cp_out[2] + cp_out[3])
        cp_patch = [copy(pbuf.at[i], out_hbm.at[grp[i] >> 2, grp[i] & 3], sems.at[4 + i]) for i in range(2)]
        _start(cp_patch)
        _wait(cp_patch)

    first_step = 0
    for layer in range(2):
        last = layer == 1
        pieces = [(g, c) for g in range(NG) for c in (AT_ORDER0 if layer + g == 0 else AT_ORDER)]
        n_q = n_att = 0

        def issue_q(n):
            g, c = pieces[n]
            if layer + g > 0 or 8 <= c <= 14:
                keep_q(g, c)

        for t in range(first_step, NG * NC):
            g, s = divmod(t, NC)
            first = layer + g == 0
            if first:
                if t == X_STEPS[0]:
                    _wait([cp_x[0]] + cp_w[0])
                    stage_x(0)
                    prep_wqkv(0)
                    load_column(KV_ORDER0[0])
                    n_x, staged = 1, 4
                if t == X_STEPS[1]:
                    _start(cp_w[1] + cp_w[2] + cp_w[3] + cp_wo)
                    _wait([cp_x[3]])
                    stage_x(3)
                    staged = 8
                if t == X_STEPS[2]:
                    _wait([cp_x[2], cp_x[1]])
                    stage_x(2)
                    stage_x(1)
                    staged = 16
            if layer == 0 and t == W_STEP:
                _start(cp_ffn + cp_spare)
                _wait(cp_w[1] + cp_w[2] + cp_w[3] + cp_wo)
                for gg in range(1, NG):
                    prep_wqkv(gg)
                prep_wo()
                for gg, cc in pieces[:n_att]:
                    u = oT[cc, _rows(gg, 128), :].astype(F32) * womu[gg]
                    omean[gg, cc] = _tree(jnp.add, [u[_rows(d)] for d in range(16)])
            c = (KV_ORDER0 if first else KV_ORDER)[s]
            keep_kv(g, c, project(g, c))
            if first:
                if not 8 <= c <= 14:
                    keep_q(g, c)
                while n_x <= min(t + (1 if t + 1 in X_STEPS else 3), staged - 1):
                    load_column(KV_ORDER0[n_x])
                    n_x += 1
            while n_q <= t - LAG:
                issue_q(n_q)
                n_q += 1
            while n_att < t - LAG:
                attend(*pieces[n_att], last or t >= W_STEP)
                n_att += 1

        prev = None
        for c in range(NC + 1):
            if not last and c == FFN_COL:
                _wait(cp_ffn)
            if not last and c == NC:
                prep_ffn()
            cur = out_proj(c, last, prev[1] if c and not last else None) if c < NC else None
            if n_att < len(pieces):
                attend(*pieces[n_att], True)
                n_att += 1
            if n_q < len(pieces):
                issue_q(n_q)
                n_q += 1
            if c and last:
                emit(c - 1, prev[0], prev[1])
                if c % 4 == 0 and c < NC:
                    flush(c // 4 - 1)
                if c == 12:
                    _start(cp_out[0] + cp_out[1] + cp_out[2])
                    _wait(cp_spare)
            elif c:
                next_norm(c - 1, prev[0] * (cur[2] if cur else lax.rsqrt(prev[1] + EPS)))
            prev = cur
        first_step = route(last)


@jax.jit
def pallas_interleave_layers__sliding_local_dilated__moe_arch_mod__prompt_kernel(
        A_x, A_wqkv, A_wo, B_x, B_w_r, B_w_gate, B_w_up, B_w_down):
    del B_x
    hbm = pl.BlockSpec(memory_space=pltpu.HBM)
    vmem = pltpu.VMEM
    out = pl.pallas_call(
        _kernel,
        out_shape=jax.ShapeDtypeStruct((64, 4, 8, D), BF16),
        in_specs=[hbm] * 7,
        out_specs=hbm,
        scratch_shapes=[
            vmem((4, 64, 8, D), BF16),
            vmem((3 * NG, D, 128), BF16),
            vmem((D, D), BF16),
            vmem((D,), BF16),
            vmem((D,), BF16),
            vmem((F, D), BF16),
            vmem((F, D), BF16),
            vmem((F, D), BF16),
            vmem((64, 64, 128), U32),
            vmem((NG, 4, 384, 128), BF16),
            vmem((4, D, 128), BF16),
            vmem((NG, 128, 128), F32),
            vmem((NG, NC, 8, 128), F32),
            vmem((D, 128), F32),
            vmem((D // 2, 2 * FT * 128), U32),
            vmem((FT * 64, D), U32),
            vmem((4, 4, 256, 128), U32),
            vmem((4, 4, 256, 128), U32),
            vmem((NC, D, 128), F32),
            vmem((NC, D, 128), F32),
            vmem((NC, D, 128), BF16),
            vmem((2, NC, 128, 128), F32),
            vmem((2, NC + 7, 128, 128), F32),
            vmem((2, NC + 7, 128, 128), F32),
            vmem((2, 128, 128), F32),
            vmem((NC, D, 128), BF16),
            vmem((NC, 8, 128), F32),
            vmem((NC, 128), F32),
            vmem((NC, 128), F32),
            vmem((4, 4, 64, 8, 128), BF16),
            vmem((2, 8, D), BF16),
            pltpu.SemaphoreType.DMA((14,)),
        ],
        compiler_params=pltpu.CompilerParams(vmem_limit_bytes=100 * 1024 * 1024),
    )(A_x.reshape(64, 4, 8, D), A_wqkv, A_wo, B_w_r, B_w_gate.T, B_w_up.T, B_w_down)
    return out.reshape(1, S, D)
```

```python
import jax
import jax.numpy as jnp
from jax import lax
import jax.experimental.pallas as pl
import jax.experimental.pallas.tpu as pltpu

S, D, F = 2048, 512, 1376
NC = 16
NG = 4
W = 8
FT = 11
EPS = 1e-5
SCALE = 0.25
F32, BF16, I32, U32 = jnp.float32, jnp.bfloat16, jnp.int32, jnp.uint32
NN = (((1,), (0,)), ((), ()))
NT = (((1,), (1,)), ((), ()))
K_, V_, Q_ = 0, 1, 2

KV_ORDER = [0] + list(range(9, 16)) + list(range(1, 9))
AT_ORDER = list(range(16))
KV_ORDER0 = [0, 1, 2, 3, 12, 13, 14, 15, 11, 10, 9, 8, 4, 5, 6, 7]
AT_ORDER0 = [3, 2, 1, 0, 15, 4, 5, 6, 7, 8, 9, 10, 11, 12, 13, 14]
LAG = 7
X_STEPS = (0, 2, 7)
W_STEP = 15
FFN_COL = 14
RUN_AHEAD = (3, 1, 1, 3)


def _dot(a, b, dn=NN):
    return lax.dot_general(a, b, dn, preferred_element_type=F32)


def _bf(words):
    return pltpu.bitcast(words, BF16)


def _rows(i, n=8):
    return slice(i * n, (i + 1) * n)


def _tree(op, xs):
    while len(xs) > 1:
        xs = [op(xs[i], xs[i + 1]) for i in range(0, len(xs), 2)]
    return xs[0]


def _tiles(x):
    return x.reshape(x.shape[0] // 8, 8, 128)


def _fold(x):
    return jnp.sum(_tiles(x), axis=0)


def _row_sum(x, chains=1):
    n = 8 * chains
    return jnp.sum(jnp.sum(x.reshape(x.shape[0] // n, n, 128), axis=0), axis=0, keepdims=True)


def _start(copies):
    for c in copies:
        c.start()


def _wait(copies):
    for c in copies:
        c.wait()


def _kernel(x_hbm, wqkv_hbm, wo_hbm, wr_hbm, wg_hbm, wu_hbm, wd_hbm, out_hbm,
            xin, wqkv, wo, wr, wr_spare, wg, wu, wd,
            wtmp, womu, omean, wrB, wgu, wdn, tin, tout,
            xa, xb, qT, kT, vT, v0T, stat, hscale, rstd, score, obuf, pbuf, sems):
    copy = pltpu.make_async_copy
    cp_w = [[copy(wqkv_hbm.at[:, _rows(p * NG + g, 128)], wqkv.at[p * NG + g], sems.at[g])
             for p in range(3)] for g in range(NG)]
    cp_x = [copy(x_hbm.at[:, a], xin.at[a], sems.at[4 + a]) for a in range(4)]
    cp_wo = [copy(wo_hbm, wo, sems.at[8]), copy(wr_hbm, wr, sems.at[9])]
    cp_ffn = [copy(wg_hbm, wg, sems.at[10]), copy(wu_hbm, wu, sems.at[11]), copy(wd_hbm, wd, sems.at[12])]
    cp_spare = [copy(wr_hbm, wr_spare, sems.at[13])]
    cp_out = [[copy(obuf.at[a, j], out_hbm.at[:, a, :, _rows(j, 128)], sems.at[a])
               for j in range(4)] for a in range(4)]
    _start([cp_x[0]] + cp_w[0] + [cp_x[3], cp_x[2], cp_x[1]])

    lane = lax.broadcasted_iota(I32, (8, 128), 1)
    sub = lax.broadcasted_iota(I32, (8, 128), 0)

    lane128 = lax.broadcasted_iota(I32, (128, 128), 1)

    def put(view, val):
        pltpu.store(view, val, mask=lax.broadcasted_iota(I32, val.shape, 1) >= 0)

    wT, woT, hT, oT = {}, [], {}, {}

    def channel_major(slot, t):
        wtmp[slot] = pltpu.bitcast(t, U32)
        out = []
        for i in range(8):
            u = wtmp[slot, pl.ds(i, 8, stride=8), :]
            out += [pltpu.bitcast(u << 16, F32), pltpu.bitcast((u >> 16) << 16, F32)]
        return jnp.concatenate(out, axis=0)

    def prep_wqkv(g):
        w = {}
        for p, part in enumerate((Q_, K_, V_)):
            t = wqkv[p * NG + g].T
            t = jnp.concatenate([channel_major(16 + 12 * g + 4 * p + j, t[:, _rows(j, 128)])
                                 for j in range(4)], axis=1)
            w[part] = t * SCALE if part == Q_ else t
        wT[g, Q_] = w[Q_].astype(BF16)
        wT[g, K_] = jnp.concatenate([w[K_], w[V_]], axis=0).astype(BF16)

    def prep_wo():
        wrB[...] = jnp.broadcast_to(wr[...].astype(F32).reshape(1, D), (128, D)).T
        for g in range(NG):
            t = [channel_major(4 * g + j, wo[_rows(g, 128), _rows(j, 128)]) for j in range(4)]
            mu = jnp.sum(_tree(jnp.add, t), axis=1, keepdims=True) * (1.0 / D)
            woT.append(jnp.concatenate([u - mu for u in t], axis=1))
            womu[g] = jnp.broadcast_to(mu, (128, 128))
        woT[:] = [jnp.concatenate(woT, axis=0).astype(BF16).T]

    def prep_ffn():
        for t in range(FT):
            n = min(128, F - t * 128)
            for i, w in enumerate((wg, wu)):
                a = w[t * 128:t * 128 + n, :]
                if n < 128:
                    a = jnp.concatenate([a, jnp.zeros((128 - n, D), BF16)], axis=0)
                wgu[:, _rows(2 * t + i, 128)] = pltpu.bitcast(a.T, U32)
            wdn[t * 64:t * 64 + n // 2, :] = pltpu.bitcast(wd[t * 128:t * 128 + n, :], U32)
        wdn[F // 2:, :] = jnp.zeros((FT * 64 - F // 2, D), U32)

    def norm_column(c, x, mean0, dst):
        m = _row_sum(x, 4) * (1.0 / D)
        x = x - m
        put(dst.at[c], x)
        var = _row_sum(x * x, 4) * (1.0 / D)
        stat[c] = jnp.where(sub == 0, m if mean0 is None else mean0 + m, 1.0)
        hscale[pl.ds(c, 1), :] = lax.rsqrt(var + EPS)

    def normed(c, src):
        return (src[c] * hscale[pl.ds(c, 1), :]).astype(BF16)

    def stage_x(a):
        for j in range(4):
            tin[a, j] = pltpu.bitcast(xin[a, :, :, _rows(j, 128)].reshape(512, 128), U32)

    def load_column(c):
        x = [_bf(tin[c // 4, j, pl.ds(c % 4, 64, stride=4), :]).T.astype(F32) for j in range(4)]
        norm_column(c, jnp.concatenate(x, axis=0), None, xa)
        hT[c] = normed(c, xa)

    def keep_kv(g, c, r):
        b = g % 2
        k, v = r[_rows(K_, 128)], r[_rows(V_, 128)]
        put(kT.at[b, c + 7], k)
        if c >= 9:
            put(kT.at[b, c - 9], pltpu.roll(k, 2, 1))
        put(vT.at[b, c + 7], v)
        if c == 0:
            v0T[b] = jnp.where(lane128 == 0, v, pltpu.roll(v, 1, 1))
        if c >= 9:
            put(vT.at[b, c - 9], jnp.where(lane128 < 2, v0T[b], pltpu.roll(v, 2, 1)))

    def keep_q(g, c):
        qT[g % 2, c] = _dot(wT[g, Q_], hT[c])

    def attend(g, c, with_mean):
        b = g % 2
        q = qT[b, c]
        logit = [_fold(q * kT[b, c + 7 - w]) for w in range(W)]
        for w in range(c + 1, W):
            logit[w] = jnp.where(lane < 2, -1e9, logit[w])
        top = _tree(jnp.maximum, logit)
        e = [jnp.exp(a - top) for a in logit]
        inv = 1.0 / _tree(jnp.add, e)
        o = e[0] * _tiles(vT[b, c + 7])
        for w in range(1, W):
            o = o + e[w] * _tiles(vT[b, c + 7 - w])
        o = (o * inv).reshape(128, 128)
        oT[g, c] = o.astype(BF16)
        if with_mean:
            omean[g, c] = _fold(o * womu[g])

    def out_proj(c, last, pending):
        r = _dot(woT[0], jnp.concatenate([oT[g, c] for g in range(NG)], axis=0))
        st = stat[c]
        if last:
            x = xb[c] * st[1:2] + r
            xa[c] = x
        else:
            x = xa[c] + r
            xb[c] = x
        var = _row_sum(x * x, 2) * (1.0 / D)
        shift = _tree(jnp.add, [omean[g, c] for g in range(NG)])
        mean = st[0:1] + jnp.sum(shift, axis=0, keepdims=True)
        if pending is None:
            rs = lax.rsqrt(var + EPS)
        else:
            both = lax.rsqrt(jnp.where(sub == 0, var, pending) + EPS)
            rs, pending = both[0:1], both[1:2]
        score[pl.ds(c, 1), :] = _row_sum(x * wrB[...]) * rs
        rstd[pl.ds(c, 1), :] = rs
        gain = 1.0 + rs
        if last:
            return gain, mean, None
        stat[c] = jnp.where(sub == 0, mean, gain)
        return gain, var * gain * gain, pending

    def emit(c, gain, mean):
        for j in range(4):
            x = xa[c, _rows(j, 128), :] * gain + mean
            tout[c // 4, j, pl.ds(c % 4, 64, stride=4), :] = pltpu.bitcast(x.astype(BF16).T, U32)

    def flush(a):
        for j in range(4):
            obuf[a, j] = _bf(tout[a, j]).reshape(64, 8, 128)

    def route(last):
        early = {}

        def run_ahead(n):
            for _ in range(0 if last else n):
                c = KV_ORDER[len(early)]
                early[c] = _dot(wT[0, K_], normed(c, xb))

        r = score[...]
        cc = lax.broadcasted_iota(I32, (NC, 128), 0)
        ll = lax.broadcasted_iota(I32, (NC, 128), 1)
        pos = (ll // 2) * 32 + 2 * cc + ll % 2
        neg = jnp.logical_not(r >= 0.0)
        mag = jnp.clip(pltpu.bitcast(r, I32) & 0x7FFFFFFF, 0x00800000, 0x7F7FFFFF) & ~(S - 1)
        key = pltpu.bitcast(mag | jnp.where(neg, pos, S - 1 - pos), F32)
        key = jnp.where(neg, -key, key)
        k0 = jnp.max(key, keepdims=True)
        k1 = jnp.max(jnp.where(key == k0, -jnp.inf, key), keepdims=True)
        idx = []
        for k in (k0, k1):
            low = pltpu.bitcast(jnp.broadcast_to(k, (8, 128)), I32) & (S - 1)
            idx.append(jnp.where(k < 0.0, low, S - 1 - low)[0, 0])
        cs = [(p >> 1) & (NC - 1) for p in idx]
        ls = [((p >> 5) << 1) | (p & 1) for p in idx]
        rsel = [jnp.sum(jnp.where(lane[0:1] == ls[i], score[pl.ds(cs[i], 1), :], 0.0), keepdims=True)
                for i in range(2)]

        row = lax.broadcasted_iota(I32, (16, 128), 0)
        lanes = lax.broadcasted_iota(I32, (D, 128), 1)
        run_ahead(RUN_AHEAD[0])
        sel = []
        for i in range(2):
            h = (xa if last else xb)[cs[i]] * rstd[pl.ds(cs[i], 1), :]
            h = jnp.where(lanes == ls[i], h, 0.0).astype(BF16)
            sel.append(_dot(jnp.where(row == i, 1.0, 0.0).astype(BF16), h, NT))
        sel = jnp.where(lax.broadcasted_iota(I32, (16, D), 0) == 0, sel[0], sel[1]).astype(BF16)
        if last:
            flush(3)
            _start(cp_out[3])
            _wait(cp_out[0])
        run_ahead(RUN_AHEAD[1])
        gu = _dot(sel, _bf(wgu[...]))[0:8]
        act = []
        for t in range(FT):
            gate = gu[:, _rows(2 * t, 128)]
            act.append(gate * jax.nn.sigmoid(gate) * gu[:, _rows(2 * t + 1, 128)])
        act = jnp.concatenate(act, axis=1)
        act = jnp.concatenate([act, jnp.zeros_like(act)], axis=0).astype(BF16)
        run_ahead(RUN_AHEAD[2])
        y = _dot(act, _bf(wdn[...]))
        run_ahead(RUN_AHEAD[3])
        ys = [y[i:i + 1, :] * jax.nn.sigmoid(rsel[i]) for i in range(2)]

        if not last:
            for i in range(2):
                upd = jnp.broadcast_to(ys[i], (128, D)).astype(BF16).T.astype(F32)
                st = stat[cs[i]]
                x = xb[cs[i]] * st[1:2]
                x = jnp.where(lanes == ls[i], x + upd, x)
                norm_column(cs[i], x, st[0:1], xb)
            redo = [_dot(wT[0, K_], normed(cs[i], xb)) for i in range(2)]
            for c in KV_ORDER:
                hT[c] = normed(c, xb)
            for c, r in early.items():
                keep_kv(0, c, jnp.where(cs[0] == c, redo[0], jnp.where(cs[1] == c, redo[1], r)))
            return len(early)

        grp = [p >> 3 for p in idx]
        grp[1] = jnp.where(grp[0] == grp[1], grp[0] ^ 1, grp[1])
        for i in range(2):
            for j in range(4):
                t = obuf[grp[i] & 3, j, grp[i] >> 2].astype(F32)
                for k in range(2):
                    t = jnp.where(sub + grp[i] * 8 == idx[k], t + ys[k][:, _rows(j, 128)], t)
                pbuf[i, :, _rows(j, 128)] = t.astype(BF16)
        _wait(cp_out[1] + cp_out[2] + cp_out[3])
        cp_patch = [copy(pbuf.at[i], out_hbm.at[grp[i] >> 2, grp[i] & 3], sems.at[4 + i]) for i in range(2)]
        _start(cp_patch)
        _wait(cp_patch)

    first_step = 0
    for layer in range(2):
        last = layer == 1
        pieces = [(g, c) for g in range(NG) for c in (AT_ORDER0 if layer + g == 0 else AT_ORDER)]
        n_q = n_att = 0

        def issue_q(n):
            g, c = pieces[n]
            if layer + g > 0 or 8 <= c <= 14:
                keep_q(g, c)

        for t in range(first_step, NG * NC):
            g, s = divmod(t, NC)
            first = layer + g == 0
            if first:
                if t == X_STEPS[0]:
                    _wait([cp_x[0]] + cp_w[0])
                    stage_x(0)
                    prep_wqkv(0)
                    load_column(KV_ORDER0[0])
                    n_x, staged = 1, 4
                if t == X_STEPS[1]:
                    _start(cp_w[1] + cp_w[2] + cp_w[3] + cp_wo)
                    _wait([cp_x[3]])
                    stage_x(3)
                    staged = 8
                if t == X_STEPS[2]:
                    _wait([cp_x[2], cp_x[1]])
                    stage_x(2)
                    stage_x(1)
                    staged = 16
            if layer == 0 and t == W_STEP:
                _start(cp_ffn + cp_spare)
                _wait(cp_w[1] + cp_w[2] + cp_w[3] + cp_wo)
                for gg in range(1, NG):
                    prep_wqkv(gg)
                prep_wo()
                for gg, cc in pieces[:n_att]:
                    omean[gg, cc] = _fold(oT[gg, cc].astype(F32) * womu[gg])
            c = (KV_ORDER0 if first else KV_ORDER)[s]
            keep_kv(g, c, _dot(wT[g, K_], hT[c]))
            if first:
                if not 8 <= c <= 14:
                    keep_q(g, c)
                while n_x <= min(t + (1 if t + 1 in X_STEPS else 3), staged - 1):
                    load_column(KV_ORDER0[n_x])
                    n_x += 1
            while n_q <= t - LAG:
                issue_q(n_q)
                n_q += 1
            while n_att < t - LAG:
                attend(*pieces[n_att], last or t >= W_STEP)
                n_att += 1

        prev = None
        for c in range(NC + 1):
            if not last and c == FFN_COL:
                _wait(cp_ffn)
            if not last and c == NC:
                prep_ffn()
            cur = out_proj(c, last, prev[1] if c and not last else None) if c < NC else None
            if n_att < len(pieces):
                attend(*pieces[n_att], True)
                n_att += 1
            if n_q < len(pieces):
                issue_q(n_q)
                n_q += 1
            if c and last:
                emit(c - 1, prev[0], prev[1])
                if c % 4 == 0 and c < NC:
                    flush(c // 4 - 1)
                if c == 12:
                    _start(cp_out[0] + cp_out[1] + cp_out[2])
                    _wait(cp_spare)
            elif c:
                hscale[pl.ds(c - 1, 1), :] = prev[0] * (cur[2] if cur else lax.rsqrt(prev[1] + EPS))
            prev = cur
        first_step = route(last)


@jax.jit
def pallas_interleave_layers__sliding_local_dilated__moe_arch_mod__prompt_kernel(
        A_x, A_wqkv, A_wo, B_x, B_w_r, B_w_gate, B_w_up, B_w_down):
    del B_x
    hbm = pl.BlockSpec(memory_space=pltpu.HBM)
    vmem = pltpu.VMEM
    out = pl.pallas_call(
        _kernel,
        out_shape=jax.ShapeDtypeStruct((64, 4, 8, D), BF16),
        in_specs=[hbm] * 7,
        out_specs=hbm,
        scratch_shapes=[
            vmem((4, 64, 8, D), BF16),
            vmem((3 * NG, D, 128), BF16),
            vmem((D, D), BF16),
            vmem((D,), BF16),
            vmem((D,), BF16),
            vmem((F, D), BF16),
            vmem((F, D), BF16),
            vmem((F, D), BF16),
            vmem((64, 64, 128), U32),
            vmem((NG, 128, 128), F32),
            vmem((NG, NC, 8, 128), F32),
            vmem((D, 128), F32),
            vmem((D // 2, 2 * FT * 128), U32),
            vmem((FT * 64, D), U32),
            vmem((4, 4, 256, 128), U32),
            vmem((4, 4, 256, 128), U32),
            vmem((NC, D, 128), F32),
            vmem((NC, D, 128), F32),
            vmem((2, NC, 128, 128), F32),
            vmem((2, NC + 7, 128, 128), F32),
            vmem((2, NC + 7, 128, 128), F32),
            vmem((2, 128, 128), F32),
            vmem((NC, 8, 128), F32),
            vmem((NC, 128), F32),
            vmem((NC, 128), F32),
            vmem((NC, 128), F32),
            vmem((4, 4, 64, 8, 128), BF16),
            vmem((2, 8, D), BF16),
            pltpu.SemaphoreType.DMA((14,)),
        ],
        compiler_params=pltpu.CompilerParams(vmem_limit_bytes=100 * 1024 * 1024),
    )(A_x.reshape(64, 4, 8, D), A_wqkv, A_wo, B_w_r, B_w_gate.T, B_w_up.T, B_w_down)
    return out.reshape(1, S, D)
```
